```python
import jax
import jax.numpy as jnp

def _softmax(x, axis=-1):
    return jax.nn.softmax(x, axis=axis)
def _gelu(x):
    return jax.nn.gelu(x, approximate=True)
def _silu(x):
    return jax.nn.silu(x)
def _sigmoid(x):
    return jax.nn.sigmoid(x)
def _layernorm(x, axis=-1, eps=1e-5):
    m = jnp.mean(x, axis=axis, keepdims=True)
    v = jnp.var(x, axis=axis, keepdims=True)
    return (x - m) / jnp.sqrt(v + eps)
def _scatter_add(tgt, idx, src, axis=0):
    return tgt.at[idx].add(src)
def _segment_sum(src, seg, n):
    return jax.ops.segment_sum(src, seg, n)
class _Rng:
    def __init__(self, key):
        self._k = key
    def _next(self):
        self._k, sub = jax.random.split(self._k)
        return sub
    def normal(self, shape):
        return jax.random.normal(self._next(), shape, dtype=jnp.bfloat16)
    def randint(self, lo, hi, shape):
        return jax.random.randint(self._next(), shape, lo, hi, dtype=jnp.int32)
    def uniform(self, shape, lo=0.0, hi=1.0):
        return jax.random.uniform(self._next(), shape, jnp.bfloat16, lo, hi)
    def permutation(self, n):
        return jax.random.permutation(self._next(), n)


kernel_name = 'gated_mix__sliding_block_cached__moe_arch_mod__decode'

def setup_inputs():
    _rng = _Rng(jax.random.key(int.from_bytes(__import__("os").urandom(4), "little")))
    _w = (lambda a: (lambda t: t.astype(jnp.bfloat16) if jnp.issubdtype(t.dtype, jnp.floating) else t)(jnp.asarray(a)))
    def _A_setup():
        B, Sq, D = 1, 1, 640
        Hq, Hkv, Sk, Dh = 32, 32, 32768, 192
        assert Hq % Hkv == 0, (Hq, Hkv)
        return {
            "x": _w((lambda *s: _rng.normal(s) * 0.05)(B, Sq, D)),
            "k_cache": _w((lambda *s: _rng.normal(s) * 0.05)(B, Hkv, Sk, Dh)),
            "v_cache": _w((lambda *s: _rng.normal(s) * 0.05)(B, Hkv, Sk, Dh)),
            "wq": _w((lambda *s: _rng.normal(s) * 0.05)(D, Hq * Dh) * (D ** -0.5)),
            "wo": _w((lambda *s: _rng.normal(s) * 0.05)(Hq * Dh, D) * ((Hq * Dh) ** -0.5)),
        }
    _A_in = _A_setup()

    def _B_setup():
        B, S, D, F, C = 1, 1, 640, 1536, 1
        return {
            "x": _w((lambda *s: _rng.normal(s) * 0.05)(B, S, D)),
            "w_r": _w((lambda *s: _rng.normal(s) * 0.05)(D)),
            "w_gate": _w((lambda *s: _rng.normal(s) * 0.05)(D, F)),
            "w_up": _w((lambda *s: _rng.normal(s) * 0.05)(D, F)),
            "w_down": _w((lambda *s: _rng.normal(s) * 0.05)(F, D)),
        }
    _B_in = _B_setup()

    return {
        "A_x": _A_in["x"],
        "A_k_cache": _A_in["k_cache"],
        "A_v_cache": _A_in["v_cache"],
        "A_wq": _A_in["wq"],
        "A_wo": _A_in["wo"],
        "B_x": _B_in["x"],
        "B_w_r": _B_in["w_r"],
        "B_w_gate": _B_in["w_gate"],
        "B_w_up": _B_in["w_up"],
        "B_w_down": _B_in["w_down"],
        "gate_w": _w((lambda *s: _rng.normal(s) * 0.05)(640)),
    }

def reference(A_x, A_k_cache, A_v_cache, A_wq, A_wo, B_x, B_w_r, B_w_gate, B_w_up, B_w_down, gate_w):
    def _A_ref(x, k_cache, v_cache, wq, wo):
        B, Sq, D = x.shape
        Hq, Dh = 32, 192
        Hkv, Sk = k_cache.shape[1], k_cache.shape[2]
        W = min(4096, max(256, Sk // 4))
        rep = Hq // Hkv
        q = (lambda x, *d: x.transpose(*d))((x @ wq).reshape(B, Sq, Hq, Dh), 0, 2, 1, 3)
        k = jnp.repeat(k_cache[:, :, Sk - W:, :], rep, axis=1)
        v = jnp.repeat(v_cache[:, :, Sk - W:, :], rep, axis=1)
        scores = jnp.einsum("bhqd,bhkd->bhqk", q, k) * (Dh ** -0.5)
        p = _softmax(scores, axis=-1)
        o = jnp.einsum("bhqk,bhkd->bhqd", p, v)
        return (lambda x, *d: x.transpose(*d))(o, 0, 2, 1, 3).reshape(B, Sq, Hq * Dh) @ wo

    def _B_ref(x, w_r, w_gate, w_up, w_down):
        B, S, D = x.shape
        C = 1
        r = x @ w_r
        idx = jnp.argsort(-r, axis=-1)[:, :C]
        idx_e = jnp.repeat(idx.reshape(B, C, 1), D, axis=2)
        x_sel = jnp.take_along_axis(x, idx_e, axis=1)
        g = _silu(x_sel @ w_gate)
        u = x_sel @ w_up
        y = (g * u) @ w_down
        r_sel = _sigmoid(jnp.take_along_axis(r, idx, axis=1))
        y = y * r_sel.reshape(B, C, 1)
        b_off = (jnp.arange(B) * S).reshape(B, 1)
        flat_idx = (idx + b_off).reshape(B * C)
        zero = (x * 0.0).reshape(B * S, D)
        upd = _scatter_add(zero, flat_idx, y.reshape(B * C, D), axis=0)
        return x + upd.reshape(B, S, D)

    x = A_x
    g = _sigmoid((x * gate_w).sum(-1, keepdims=True))
    a = _A_ref(x, A_k_cache, A_v_cache, A_wq, A_wo)
    b = _B_ref(x, B_w_r, B_w_gate, B_w_up, B_w_down)
    return g * a + (1 - g) * b
```

```python
import jax
import jax.numpy as jnp
import jax.experimental.pallas as pl
import jax.experimental.pallas.tpu as pltpu

_HQ = 32
_DH = 192
_PAIR = 2 * _DH
_RING = 3
_WD_PARTS = 6


def _sigmoid(x):
    return 1.0 / (1.0 + jnp.exp(-x))


def _kernel(
    x_hbm, wr_hbm, gw_hbm, kt_hbm, vt_hbm, wq_hbm, wo_hbm, wg_hbm, wu_hbm, wd_hbm,
    o_ref,
    x_buf, wr_buf, gw_buf, k_buf, v_buf, wq_buf, wo_buf, wg_buf, wu_buf, wd_buf,
    q_buf, acc_buf,
    k_sem, v_sem, w_sem, wd_sem,
    *, win_start, win, n_pairs,
):
    d_model = x_buf.shape[-1]
    f_dim = wg_buf.shape[-1]
    wd_rows = f_dim // _WD_PARTS
    f32 = jnp.float32
    bf16 = jnp.bfloat16

    def k_copy(p, slot):
        return pltpu.make_async_copy(
            kt_hbm.at[pl.ds(p * _PAIR, _PAIR), pl.ds(win_start, win)],
            k_buf.at[slot], k_sem.at[slot])

    def v_copy(p, slot):
        return pltpu.make_async_copy(
            vt_hbm.at[pl.ds(p * _PAIR, _PAIR), pl.ds(win_start, win)],
            v_buf.at[slot], v_sem.at[slot])

    x_cp = pltpu.make_async_copy(x_hbm, x_buf, w_sem.at[0])
    wr_cp = pltpu.make_async_copy(wr_hbm, wr_buf, w_sem.at[1])
    gw_cp = pltpu.make_async_copy(gw_hbm, gw_buf, w_sem.at[2])
    wq_cp = pltpu.make_async_copy(wq_hbm, wq_buf, w_sem.at[3])
    wo_cp = pltpu.make_async_copy(wo_hbm, wo_buf, w_sem.at[4])
    wg_cp = pltpu.make_async_copy(wg_hbm, wg_buf, w_sem.at[5])
    wu_cp = pltpu.make_async_copy(wu_hbm, wu_buf, w_sem.at[6])
    wd_cps = [
        pltpu.make_async_copy(
            wd_hbm.at[pl.ds(j * wd_rows, wd_rows)],
            wd_buf.at[pl.ds(j * wd_rows, wd_rows)], wd_sem.at[j])
        for j in range(_WD_PARTS)
    ]

    x_cp.start()
    wq_cp.start()
    k_copy(0, 0).start()
    v_copy(0, 0).start()
    wo_cp.start()
    wr_cp.start()
    gw_cp.start()
    for s in range(1, _RING):
        k_copy(s, s).start()
        v_copy(s, s).start()

    x_cp.wait()
    x_row = x_buf[...]
    x8 = jnp.broadcast_to(x_row, (8, d_model))

    row = jax.lax.broadcasted_iota(jnp.int32, (8, _PAIR), 0)
    col = jax.lax.broadcasted_iota(jnp.int32, (8, _PAIR), 1)
    diag = jnp.logical_or(
        jnp.logical_and(row == 0, col < _DH),
        jnp.logical_and(row == 1, col >= _DH))

    wq_cp.wait()
    for p in range(n_pairs):
        q = jnp.dot(x8, wq_buf[:, p * _PAIR:(p + 1) * _PAIR],
                    preferred_element_type=f32)
        q_buf[p] = jnp.where(diag, q, 0.0).astype(bf16)

    acc_buf[...] = jnp.zeros_like(acc_buf)
    scale = _DH ** -0.5

    def step(p, carry):
        slot = p % _RING
        nxt = p + _RING

        k_copy(p, slot).wait()
        s = jnp.dot(q_buf[p], k_buf[slot], preferred_element_type=f32) * scale

        @pl.when(nxt < n_pairs)
        def _():
            k_copy(nxt, slot).start()

        m = jnp.max(s, axis=1, keepdims=True)
        e = jnp.exp(s - m)
        l = jnp.sum(e, axis=1, keepdims=True)

        v_copy(p, slot).wait()
        o = jax.lax.dot_general(
            e.astype(bf16), v_buf[slot], (((1,), (1,)), ((), ())),
            preferred_element_type=f32)

        @pl.when(nxt < n_pairs)
        def _():
            v_copy(nxt, slot).start()

        @pl.when(nxt == n_pairs - 1)
        def _():
            wg_cp.start()
            wu_cp.start()
            for c in wd_cps:
                c.start()

        @pl.when(p == 0)
        def _():
            wo_cp.wait()

        o = jnp.where(diag, o / l, 0.0).astype(bf16)
        acc_buf[...] += jnp.dot(o, wo_buf[p], preferred_element_type=f32)
        return carry

    jax.lax.fori_loop(0, n_pairs, step, 0)

    a = jnp.sum(acc_buf[...], axis=0, keepdims=True)

    wr_cp.wait()
    gw_cp.wait()
    xf = x_row.astype(f32)
    wr = wr_buf[...].astype(f32).reshape(1, d_model)
    gw = gw_buf[...].astype(f32).reshape(1, d_model)
    r_gate = _sigmoid(jnp.sum(xf * wr, axis=1, keepdims=True))
    g_mix = _sigmoid(jnp.sum(xf * gw, axis=1, keepdims=True))

    wg_cp.wait()
    hg = jnp.dot(x8, wg_buf[...], preferred_element_type=f32)
    wu_cp.wait()
    hu = jnp.dot(x8, wu_buf[...], preferred_element_type=f32)
    act = (hg * _sigmoid(hg) * hu).astype(bf16)

    y = jnp.zeros((8, d_model), f32)
    for j in range(_WD_PARTS):
        wd_cps[j].wait()
        y += jnp.dot(act[:, j * wd_rows:(j + 1) * wd_rows],
                     wd_buf[j * wd_rows:(j + 1) * wd_rows, :],
                     preferred_element_type=f32)
    y = y[0:1]
    b = xf + (xf * 0.0 + y * r_gate)
    o_ref[...] = (g_mix * a + (1.0 - g_mix) * b).astype(o_ref.dtype)


@jax.jit
def pallas_gated_mix__sliding_block_cached__moe_arch_mod__decode_kernel(
    A_x: jax.Array,
    A_k_cache: jax.Array,
    A_v_cache: jax.Array,
    A_wq: jax.Array,
    A_wo: jax.Array,
    B_x: jax.Array,
    B_w_r: jax.Array,
    B_w_gate: jax.Array,
    B_w_up: jax.Array,
    B_w_down: jax.Array,
    gate_w: jax.Array,
):
    del B_x
    b, sq, d_model = A_x.shape
    _, hkv, sk, dh = A_k_cache.shape
    assert (b, sq) == (1, 1) and hkv == _HQ and dh == _DH
    f_dim = B_w_gate.shape[1]
    win = min(4096, max(256, sk // 4))
    n_pairs = _HQ // 2
    assert n_pairs >= _RING and f_dim % (_WD_PARTS * 128) == 0

    kt = jnp.transpose(A_k_cache, (0, 1, 3, 2)).reshape(hkv * dh, sk)
    vt = jnp.transpose(A_v_cache, (0, 1, 3, 2)).reshape(hkv * dh, sk)
    x = A_x.reshape(1, d_model)
    wo = A_wo.reshape(n_pairs, _PAIR, d_model)

    dt = A_x.dtype
    hbm = pl.BlockSpec(memory_space=pl.ANY)
    out = pl.pallas_call(
        lambda *refs: _kernel(*refs, win_start=sk - win, win=win, n_pairs=n_pairs),
        out_shape=jax.ShapeDtypeStruct((1, d_model), dt),
        in_specs=[hbm] * 10,
        out_specs=pl.BlockSpec(memory_space=pltpu.VMEM),
        scratch_shapes=[
            pltpu.VMEM((1, d_model), dt),
            pltpu.VMEM((d_model,), dt),
            pltpu.VMEM((d_model,), dt),
            pltpu.VMEM((_RING, _PAIR, win), dt),
            pltpu.VMEM((_RING, _PAIR, win), dt),
            pltpu.VMEM((d_model, _HQ * _DH), dt),
            pltpu.VMEM((n_pairs, _PAIR, d_model), dt),
            pltpu.VMEM((d_model, f_dim), dt),
            pltpu.VMEM((d_model, f_dim), dt),
            pltpu.VMEM((f_dim, d_model), dt),
            pltpu.VMEM((n_pairs, 8, _PAIR), dt),
            pltpu.VMEM((8, d_model), jnp.float32),
            pltpu.SemaphoreType.DMA((_RING,)),
            pltpu.SemaphoreType.DMA((_RING,)),
            pltpu.SemaphoreType.DMA((7,)),
            pltpu.SemaphoreType.DMA((_WD_PARTS,)),
        ],
        compiler_params=pltpu.CompilerParams(vmem_limit_bytes=96 * 1024 * 1024),
    )(x, B_w_r, gate_w, kt, vt, A_wq, wo, B_w_gate, B_w_up, B_w_down)
    return out.reshape(b, sq, d_model)
```

```python
import jax
import jax.numpy as jnp
import jax.experimental.pallas as pl
import jax.experimental.pallas.tpu as pltpu

_HQ = 32
_DH = 192
_GROUP = 4
_ROWS = _GROUP * _DH
_N_GROUPS = _HQ // _GROUP
_RING = 2
_WD_SPLIT = (768, 384, 256, 128)


def _sigmoid(x):
    return 1.0 / (1.0 + jnp.exp(-x))


def _kernel(
    x_hbm, wr_hbm, gw_hbm, kt_hbm, vt_hbm, wq_hbm, wo_hbm, wg_hbm, wu_hbm, wd_hbm,
    o_ref,
    x_buf, wr_buf, gw_buf, k_buf, v_buf, wq_buf, wo_buf, wg_buf, wu_buf, wd_buf,
    q_buf, acc_buf,
    k_sem, v_sem, w_sem, wd_sem,
    *, win_start, win,
):
    d_model = x_buf.shape[-1]
    f32 = jnp.float32
    bf16 = jnp.bfloat16

    def k_copy(p, slot):
        return pltpu.make_async_copy(
            kt_hbm.at[pl.ds(p * _ROWS, _ROWS), pl.ds(win_start, win)],
            k_buf.at[slot], k_sem.at[slot])

    def v_copy(p, slot):
        return pltpu.make_async_copy(
            vt_hbm.at[pl.ds(p * _ROWS, _ROWS), pl.ds(win_start, win)],
            v_buf.at[slot], v_sem.at[slot])

    x_cp = pltpu.make_async_copy(x_hbm, x_buf, w_sem.at[0])
    wr_cp = pltpu.make_async_copy(wr_hbm, wr_buf, w_sem.at[1])
    gw_cp = pltpu.make_async_copy(gw_hbm, gw_buf, w_sem.at[2])
    wq_cp = pltpu.make_async_copy(wq_hbm, wq_buf, w_sem.at[3])
    wo_cp = pltpu.make_async_copy(wo_hbm, wo_buf, w_sem.at[4])
    wg_cp = pltpu.make_async_copy(wg_hbm, wg_buf, w_sem.at[5])
    wu_cp = pltpu.make_async_copy(wu_hbm, wu_buf, w_sem.at[6])
    wd_offs = [sum(_WD_SPLIT[:j]) for j in range(len(_WD_SPLIT))]
    wd_cps = [
        pltpu.make_async_copy(
            wd_hbm.at[pl.ds(o, r)], wd_buf.at[pl.ds(o, r)], wd_sem.at[j])
        for j, (o, r) in enumerate(zip(wd_offs, _WD_SPLIT))
    ]

    x_cp.start()
    wr_cp.start()
    gw_cp.start()
    wq_cp.start()
    k_copy(0, 0).start()
    v_copy(0, 0).start()
    wo_cp.start()
    for s in range(1, _RING):
        k_copy(s, s).start()
        v_copy(s, s).start()

    trailing = [[wg_cp, wu_cp]] + [[c] for c in wd_cps]
    points = [(p, w) for p in range(_N_GROUPS - _RING, _N_GROUPS) for w in "kv"]
    in_loop, after_loop = trailing[:-1], trailing[-1]
    assert len(in_loop) <= len(points)

    def start_trailing(p, which):
        for (at_p, at_which), group in zip(points, in_loop):
            if at_which == which:
                @pl.when(p == at_p)
                def _(group=group):
                    for c in group:
                        c.start()

    x_cp.wait()
    wr_cp.wait()
    gw_cp.wait()
    x_row = x_buf[...]
    x8 = jnp.broadcast_to(x_row, (8, d_model))
    xf = x_row.astype(f32)
    wr = wr_buf[...].astype(f32).reshape(1, d_model)
    gw = gw_buf[...].astype(f32).reshape(1, d_model)
    r_gate = _sigmoid(jnp.sum(xf * wr, axis=1, keepdims=True))
    g_mix = _sigmoid(jnp.sum(xf * gw, axis=1, keepdims=True))

    row = jax.lax.broadcasted_iota(jnp.int32, (8, _ROWS), 0)
    col = jax.lax.broadcasted_iota(jnp.int32, (8, _ROWS), 1)
    diag = jnp.logical_and(col >= row * _DH, col < (row + 1) * _DH)

    wq_cp.wait()
    for p in range(_N_GROUPS):
        q = jnp.dot(x8, wq_buf[:, p * _ROWS:(p + 1) * _ROWS],
                    preferred_element_type=f32)
        q_buf[p] = jnp.where(diag, q, 0.0).astype(bf16)

    acc_buf[...] = jnp.zeros_like(acc_buf)
    scale = _DH ** -0.5

    def step(p, carry):
        slot = p % _RING
        nxt = p + _RING

        k_copy(p, slot).wait()
        start_trailing(p, "k")
        s = jnp.dot(q_buf[p], k_buf[slot], preferred_element_type=f32) * scale

        @pl.when(nxt < _N_GROUPS)
        def _():
            k_copy(nxt, slot).start()

        m = jnp.max(s, axis=1, keepdims=True)
        e = jnp.exp(s - m)
        l = jnp.sum(e, axis=1, keepdims=True)

        v_copy(p, slot).wait()
        o = jax.lax.dot_general(
            e.astype(bf16), v_buf[slot], (((1,), (1,)), ((), ())),
            preferred_element_type=f32)

        @pl.when(nxt < _N_GROUPS)
        def _():
            v_copy(nxt, slot).start()

        start_trailing(p, "v")

        @pl.when(p == 0)
        def _():
            wo_cp.wait()

        o = jnp.where(diag, o / l, 0.0).astype(bf16)
        acc_buf[...] += jnp.dot(o, wo_buf[p], preferred_element_type=f32)
        return carry

    jax.lax.fori_loop(0, _N_GROUPS, step, 0)

    for c in after_loop:
        c.start()
    a = jnp.sum(acc_buf[...], axis=0, keepdims=True)

    wg_cp.wait()
    hg = jnp.dot(x8, wg_buf[...], preferred_element_type=f32)
    wu_cp.wait()
    hu = jnp.dot(x8, wu_buf[...], preferred_element_type=f32)
    act = (hg * _sigmoid(hg) * hu).astype(bf16)

    y = jnp.zeros((8, d_model), f32)
    for j, (o, r) in enumerate(zip(wd_offs, _WD_SPLIT)):
        wd_cps[j].wait()
        y += jnp.dot(act[:, o:o + r], wd_buf[o:o + r, :],
                     preferred_element_type=f32)
    b = xf + (xf * 0.0 + y[0:1] * r_gate)
    o_ref[...] = (g_mix * a + (1.0 - g_mix) * b).astype(o_ref.dtype)


@jax.jit
def pallas_gated_mix__sliding_block_cached__moe_arch_mod__decode_kernel(
    A_x: jax.Array,
    A_k_cache: jax.Array,
    A_v_cache: jax.Array,
    A_wq: jax.Array,
    A_wo: jax.Array,
    B_x: jax.Array,
    B_w_r: jax.Array,
    B_w_gate: jax.Array,
    B_w_up: jax.Array,
    B_w_down: jax.Array,
    gate_w: jax.Array,
):
    del B_x
    b, sq, d_model = A_x.shape
    _, hkv, sk, dh = A_k_cache.shape
    f_dim = B_w_gate.shape[1]
    assert (b, sq) == (1, 1) and hkv == _HQ and dh == _DH
    assert sum(_WD_SPLIT) == f_dim and _N_GROUPS > _RING
    win = min(4096, max(256, sk // 4))

    kt = jnp.transpose(A_k_cache, (0, 1, 3, 2)).reshape(hkv * dh, sk)
    vt = jnp.transpose(A_v_cache, (0, 1, 3, 2)).reshape(hkv * dh, sk)
    x = A_x.reshape(1, d_model)
    wo = A_wo.reshape(_N_GROUPS, _ROWS, d_model)

    dt = A_x.dtype
    hbm = pl.BlockSpec(memory_space=pl.ANY)
    out = pl.pallas_call(
        lambda *refs: _kernel(*refs, win_start=sk - win, win=win),
        out_shape=jax.ShapeDtypeStruct((1, d_model), dt),
        in_specs=[hbm] * 10,
        out_specs=pl.BlockSpec(memory_space=pltpu.VMEM),
        scratch_shapes=[
            pltpu.VMEM((1, d_model), dt),
            pltpu.VMEM((d_model,), dt),
            pltpu.VMEM((d_model,), dt),
            pltpu.VMEM((_RING, _ROWS, win), dt),
            pltpu.VMEM((_RING, _ROWS, win), dt),
            pltpu.VMEM((d_model, _HQ * _DH), dt),
            pltpu.VMEM((_N_GROUPS, _ROWS, d_model), dt),
            pltpu.VMEM((d_model, f_dim), dt),
            pltpu.VMEM((d_model, f_dim), dt),
            pltpu.VMEM((f_dim, d_model), dt),
            pltpu.VMEM((_N_GROUPS, 8, _ROWS), dt),
            pltpu.VMEM((8, d_model), jnp.float32),
            pltpu.SemaphoreType.DMA((_RING,)),
            pltpu.SemaphoreType.DMA((_RING,)),
            pltpu.SemaphoreType.DMA((7,)),
            pltpu.SemaphoreType.DMA((len(_WD_SPLIT),)),
        ],
        compiler_params=pltpu.CompilerParams(vmem_limit_bytes=96 * 1024 * 1024),
    )(x, B_w_r, gate_w, kt, vt, A_wq, wo, B_w_gate, B_w_up, B_w_down)
    return out.reshape(b, sq, d_model)
```
